```python
import jax
import jax.numpy as jnp

def _softmax(x, axis=-1):
    return jax.nn.softmax(x, axis=axis)

def _gelu(x):
    return jax.nn.gelu(x, approximate=True)

def _silu(x):
    return jax.nn.silu(x)

def _sigmoid(x):
    return jax.nn.sigmoid(x)

def _layernorm(x, axis=-1, eps=1e-05):
    m = jnp.mean(x, axis=axis, keepdims=True)
    v = jnp.var(x, axis=axis, keepdims=True)
    return (x - m) / jnp.sqrt(v + eps)

def _scatter_add(tgt, idx, src, axis=0):
    return tgt.at[idx].add(src)

def _segment_sum(src, seg, n):
    return jax.ops.segment_sum(src, seg, n)

class _Rng:

    def __init__(self, key):
        self._k = key

    def _next(self):
        self._k, sub = jax.random.split(self._k)
        return sub

    def normal(self, shape):
        return jax.random.normal(self._next(), shape, dtype=jnp.bfloat16)

    def randint(self, lo, hi, shape):
        return jax.random.randint(self._next(), shape, lo, hi, dtype=jnp.int32)

    def uniform(self, shape, lo=0.0, hi=1.0):
        return jax.random.uniform(self._next(), shape, jnp.bfloat16, lo, hi)

    def permutation(self, n):
        return jax.random.permutation(self._next(), n)
kernel_name = 'adaLN_cond__gqa_block_cached__moe_arch_mod__prompt'

def setup_inputs():
    _rng = _Rng(jax.random.key(int.from_bytes(__import__("os").urandom(4), "little")))
    _w = lambda a: (lambda t: t.astype(jnp.bfloat16) if jnp.issubdtype(t.dtype, jnp.floating) else t)(jnp.asarray(a))

    def _A_setup():
        B, Sq, D = (1, 2048, 576)
        Hq, Hkv, Sk, Dh = (32, 16, 2048, 128)
        assert Hq % Hkv == 0, (Hq, Hkv)
        return {'x': _w((lambda *s: _rng.normal(s) * 0.05)(B, Sq, D)), 'k_cache': _w((lambda *s: _rng.normal(s) * 0.05)(B, Hkv, Sk, Dh)), 'v_cache': _w((lambda *s: _rng.normal(s) * 0.05)(B, Hkv, Sk, Dh)), 'wq': _w((lambda *s: _rng.normal(s) * 0.05)(D, Hq * Dh) * D ** (-0.5)), 'wo': _w((lambda *s: _rng.normal(s) * 0.05)(Hq * Dh, D) * (Hq * Dh) ** (-0.5))}
    _A_in = _A_setup()

    def _B_setup():
        B, S, D, F, C = (1, 2048, 576, 4608, 8)
        return {'x': _w((lambda *s: _rng.normal(s) * 0.05)(B, S, D)), 'w_r': _w((lambda *s: _rng.normal(s) * 0.05)(D)), 'w_gate': _w((lambda *s: _rng.normal(s) * 0.05)(D, F)), 'w_up': _w((lambda *s: _rng.normal(s) * 0.05)(D, F)), 'w_down': _w((lambda *s: _rng.normal(s) * 0.05)(F, D))}
    _B_in = _B_setup()
    return {'A_x': _A_in['x'], 'A_k_cache': _A_in['k_cache'], 'A_v_cache': _A_in['v_cache'], 'A_wq': _A_in['wq'], 'A_wo': _A_in['wo'], 'B_x': _B_in['x'], 'B_w_r': _B_in['w_r'], 'B_w_gate': _B_in['w_gate'], 'B_w_up': _B_in['w_up'], 'B_w_down': _B_in['w_down'], 'c': _w((lambda *s: _rng.normal(s) * 0.05)(1, 576)), 'w_mod': _w((lambda *s: _rng.normal(s) * 0.05)(576, 6 * 576) * 576 ** (-0.5))}

def reference(A_x, A_k_cache, A_v_cache, A_wq, A_wo, B_x, B_w_r, B_w_gate, B_w_up, B_w_down, c, w_mod):

    def _A_ref(x, k_cache, v_cache, wq, wo):
        B, Sq, D = x.shape
        Hq, Dh = (32, 128)
        Hkv = k_cache.shape[1]
        rep = Hq // Hkv
        q = (lambda x, *d: x.transpose(*d))((x @ wq).reshape(B, Sq, Hq, Dh), 0, 2, 1, 3)
        k = jnp.repeat(k_cache, rep, axis=1)
        v = jnp.repeat(v_cache, rep, axis=1)
        scores = jnp.einsum('bhqd,bhkd->bhqk', q, k) * Dh ** (-0.5)
        p = _softmax(scores, axis=-1)
        o = jnp.einsum('bhqk,bhkd->bhqd', p, v)
        return (lambda x, *d: x.transpose(*d))(o, 0, 2, 1, 3).reshape(B, Sq, Hq * Dh) @ wo

    def _B_ref(x, w_r, w_gate, w_up, w_down):
        B, S, D = x.shape
        C = 8
        r = x @ w_r
        idx = jnp.argsort(-r, axis=-1)[:, :C]
        idx_e = jnp.repeat(idx.reshape(B, C, 1), D, axis=2)
        x_sel = jnp.take_along_axis(x, idx_e, axis=1)
        g = _silu(x_sel @ w_gate)
        u = x_sel @ w_up
        y = g * u @ w_down
        r_sel = _sigmoid(jnp.take_along_axis(r, idx, axis=1))
        y = y * r_sel.reshape(B, C, 1)
        b_off = (jnp.arange(B) * S).reshape(B, 1)
        flat_idx = (idx + b_off).reshape(B * C)
        zero = (x * 0.0).reshape(B * S, D)
        upd = _scatter_add(zero, flat_idx, y.reshape(B * C, D), axis=0)
        return x + upd.reshape(B, S, D)
    x = A_x
    mod = (_silu(c) @ w_mod).reshape(c.shape[0], 6, 1, -1)
    sa, ca, ga, sb, cb, gb = (mod[:, 0].copy(), mod[:, 1].copy(), mod[:, 2].copy(), mod[:, 3].copy(), mod[:, 4].copy(), mod[:, 5].copy())
    h = _layernorm(x, axis=-1) * (1 + ca) + sa
    x = x + ga * _A_ref(h, A_k_cache, A_v_cache, A_wq, A_wo)
    h = _layernorm(x, axis=-1) * (1 + cb) + sb
    x = x + gb * _B_ref(h, B_w_r, B_w_gate, B_w_up, B_w_down)
    return x
```

```python
import jax
import jax.numpy as jnp
from jax import lax
from jax.experimental import pallas as pl
from jax.experimental.pallas import tpu as pltpu

HQ, DH = 32, 128
TOPC = 8
EPS = 1e-5
LOG2E = 1.4426950408889634
LANES = 128

F32 = jnp.float32
BF16 = jnp.bfloat16
U32 = jnp.uint32


def _r(x):
    return x.astype(BF16).astype(F32)


def _nt(a, b):
    return lax.dot_general(a, b, (((1,), (1,)), ((), ())), preferred_element_type=F32)


def _mm(a, b):
    return jnp.dot(a, b, preferred_element_type=F32)


def _pack(a, b):
    return pltpu.pack_elementwise([a, b], packed_dtype=BF16)


def _pack16(x):
    parts = [_pack(x[16 * i:16 * i + 8], x[16 * i + 8:16 * i + 16]) for i in range(x.shape[0] // 16)]
    return parts[0] if len(parts) == 1 else jnp.concatenate(parts, axis=0)


def _bf(x):
    return pltpu.bitcast(x, BF16)


def _recip(l):
    r = pl.reciprocal(l, approx=True)
    return r * (2.0 - l * r)


def _order(nblk):
    o = ['A0', 'B0', 'O']
    for j in range(1, nblk):
        o += [f'A{j}', f'B{j}', f'C{j-1}']
    return o + ['Q', f'C{nblk-1}']


def _make_kernel(S, D, HKV, SK, F, BQ, XCH, lnu):
    REP = HQ // HKV
    NB = S // BQ
    T = HKV * NB
    NT = S // LANES
    MQ = 128
    KR = 512
    NR = SK // KR
    NKT = SK // LANES
    DM = D // LANES * LANES
    blocks = [(r, b) for r in range(REP) for b in range(BQ // MQ)]
    NBLK = len(blocks)
    order = _order(NBLK)
    WA = 2 * D // LANES
    assert (2 * D) % LANES == 0 and NT % XCH == 0
    TPC = NT // XCH

    def kernel(xT_hbm, k_hbm, v_hbm, wq_hbm, woT_hbm, wr_ref, wg_hbm, wu_hbm, wdT_hbm, c_ref, wm_hbm,
               oT_hbm,
               xT_v, k_v, v_v, wq_v, woT_v, wg_v, wu_v, wdT_v, wm_v,
               h_v, q_v, ao_v, accT_v, col_v, h2T_v, r_v, oh_v,
               sem_x, sem_wm, sem_g, sem_moe, sem_o, *sp):
        s_v = sp[:NBLK]
        p_v = sp[NBLK:2 * NBLK]
        m_v = sp[2 * NBLK:3 * NBLK]
        ku_v = k_v.bitcast(U32)
        vu_v = v_v.bitcast(U32)
        wqu_v = wq_v.bitcast(U32)
        wou_v = woT_v.bitcast(U32)

        def grp_copies(g, sem):
            cps = []
            for r in range(REP):
                hh = g * REP + r
                c0 = pl.multiple_of(hh * DH, DH)
                cps.append(pltpu.make_async_copy(wq_hbm.at[:, pl.ds(c0, DH)], wq_v.at[hh], sem))
            cps.append(pltpu.make_async_copy(k_hbm.at[g], k_v.at[g], sem))
            cps.append(pltpu.make_async_copy(v_hbm.at[g], v_v.at[g], sem))
            for r in range(REP):
                hh = g * REP + r
                c0 = pl.multiple_of(hh * DH, DH)
                cps.append(pltpu.make_async_copy(woT_hbm.at[:, pl.ds(c0, DH)], woT_v.at[hh], sem))
            return cps

        def x_copies(ch):
            return [pltpu.make_async_copy(xT_hbm.at[:, pl.ds(i * LANES, LANES)], xT_v.at[i], sem_x.at[ch])
                    for i in range(ch * TPC, (ch + 1) * TPC)]

        def o_copies(ch):
            return [pltpu.make_async_copy(xT_v.at[i], oT_hbm.at[:, pl.ds(i * LANES, LANES)], sem_o)
                    for i in range(ch * TPC, (ch + 1) * TPC)]

        cp_wm = (
            pltpu.make_async_copy(wm_hbm.at[:, pl.ds(0, 2 * D)], wm_v.at[:, pl.ds(0, 2 * D)], sem_wm.at[0]),
            pltpu.make_async_copy(wm_hbm.at[:, pl.ds(2 * D, 4 * D)], wm_v.at[:, pl.ds(2 * D, 4 * D)], sem_wm.at[1]),
        )
        cp_moe = (
            pltpu.make_async_copy(wg_hbm, wg_v, sem_moe),
            pltpu.make_async_copy(wu_hbm, wu_v, sem_moe),
            pltpu.make_async_copy(wdT_hbm, wdT_v, sem_moe),
        )

        cp_wm[0].start()
        for cp in x_copies(0):
            cp.start()
        for cp in grp_copies(0, sem_g.at[0]):
            cp.start()
        for ch in range(1, XCH):
            for cp in x_copies(ch):
                cp.start()

        def z_body(i, _):
            accT_v[i] = jnp.zeros((D, LANES), F32)
            return _
        lax.fori_loop(0, NT, z_body, None)
        ao_v[1] = jnp.zeros((REP, BQ // 2, DH), U32)

        cf = c_ref[...].astype(F32)
        sc = _r(cf * _r(jax.nn.sigmoid(cf))).astype(BF16)
        sc8 = jnp.broadcast_to(sc, (8, D))
        cp_wm[0].wait()
        mod_a = _r(_mm(sc8, wm_v[:, 0:2 * D]))[0:1]
        sa = mod_a[:, 0:D]
        ca1 = _r(1.0 + mod_a[:, D:2 * D])

        eye = (lax.broadcasted_iota(jnp.int32, (LANES, LANES), 0)
               == lax.broadcasted_iota(jnp.int32, (LANES, LANES), 1)).astype(BF16)

        def ln1_tile(i):
            x = xT_v[i].astype(F32)
            xc = x - jnp.sum(x, axis=0, keepdims=True) * (1.0 / D)
            var = jnp.sum(xc * xc, axis=0, keepdims=True) * (1.0 / D)
            xh = (xc * lax.rsqrt(var + EPS)).astype(BF16)
            xn = _nt(eye, xh)
            h_v[pl.ds(pl.multiple_of(i * (LANES // 2), LANES // 2), LANES // 2), :] = \
                _pack16(_r(xn * ca1) + sa)

        for ch in range(XCH):
            for cp in x_copies(ch):
                cp.wait()
            if ch == 1:
                for cp in grp_copies(1, sem_g.at[1]):
                    cp.start()
                cp_wm[1].start()
            for i in range(ch * TPC, (ch + 1) * TPC):
                ln1_tile(i)

        qscale = LOG2E * DH ** -0.5

        def attn_pieces(t, slot, zero):
            g = t // NB

            def a_step(j):
                def f():
                    r, b = blocks[j]
                    q = _bf(q_v[slot, r, b * (MQ // 2):(b + 1) * (MQ // 2), :])
                    mp = None
                    for rd in range(NR):
                        s = _nt(q, _bf(ku_v[g, rd * (KR // 2):(rd + 1) * (KR // 2), :]))
                        s_v[j][0, :, rd * KR:(rd + 1) * KR] = s
                        for n in range(KR // LANES):
                            sn = s[:, n * LANES:(n + 1) * LANES]
                            mp = sn if mp is None else jnp.maximum(mp, sn)
                    m_v[j][0] = jnp.broadcast_to(jnp.max(mp, axis=1, keepdims=True), (MQ, LANES))
                return f

            def b_step(j):
                def f():
                    chain = None
                    for c in range(MQ // 16):
                        ra = slice(c * 16, c * 16 + 8)
                        rb = slice(c * 16 + 8, c * 16 + 16)
                        ma = m_v[j][zero, ra, :]
                        mb = m_v[j][zero, rb, :]
                        if chain is not None:
                            ma = jnp.maximum(ma, jnp.minimum(chain[0], ma))
                            mb = jnp.maximum(mb, jnp.minimum(chain[1], mb))
                        la = lb = None
                        for n in range(NKT):
                            cols = slice(n * LANES, (n + 1) * LANES)
                            pa = jnp.exp2(s_v[j][zero, ra, cols] - ma)
                            pb = jnp.exp2(s_v[j][zero, rb, cols] - mb)
                            p_v[j][0, n, c * 8:c * 8 + 8, :] = _pack(pa, pb)
                            la = pa if la is None else la + pa
                            lb = pb if lb is None else lb + pb
                        chain = (la, lb)
                        base = 16 * (c % 4)
                        lp = NKT + c // 4
                        p_v[j][0, lp, pl.ds(base, 8, stride=2), :] = pltpu.bitcast(
                            jnp.broadcast_to(jnp.sum(la, axis=1, keepdims=True), (8, LANES)), U32)
                        p_v[j][0, lp, pl.ds(base + 1, 8, stride=2), :] = pltpu.bitcast(
                            jnp.broadcast_to(jnp.sum(lb, axis=1, keepdims=True), (8, LANES)), U32)
                return f

            def c_step(j):
                def f():
                    r, b = blocks[j]
                    o = None
                    for rd in range(NR):
                        pp = _bf(jnp.concatenate(
                            [p_v[j][zero, rd * (KR // LANES) + n] for n in range(KR // LANES)], axis=1))
                        part = _mm(pp, _bf(vu_v[g, rd * (KR // 2):(rd + 1) * (KR // 2), :]))
                        o = part if o is None else o + part
                    l = jnp.concatenate([pltpu.bitcast(p_v[j][zero, NKT + c], F32) for c in range(2)], axis=0)
                    ao_v[slot, r, b * (MQ // 2):(b + 1) * (MQ // 2), :] = _pack16(o * _recip(l))
                return f

            pieces = {}
            for j in range(NBLK):
                pieces[f'A{j}'] = a_step(j)
                pieces[f'B{j}'] = b_step(j)
                pieces[f'C{j}'] = c_step(j)
            return pieces

        def qproj(t, slot):
            g = t // NB
            i = t % NB
            rows = pl.ds(pl.multiple_of(i * (BQ // 2), BQ // 2), BQ // 2)
            hm = _bf(h_v[rows, 0:DM])
            mains = [_mm(hm, _bf(wqu_v[g * REP + r, 0:DM // 2, :])) for r in range(REP)]
            for r in range(REP):
                wt = _bf(wqu_v[g * REP + r, DM // 2:D // 2, :])
                for b in range(BQ // MQ):
                    rws = pl.ds(pl.multiple_of(i * (BQ // 2) + b * (MQ // 2), MQ // 2), MQ // 2)
                    qq = mains[r][b * MQ:(b + 1) * MQ] + _mm(_bf(h_v[rws, DM:D]), wt)
                    q_v[slot, r, b * (MQ // 2):(b + 1) * (MQ // 2), :] = _pack16(qq * qscale)

        def oproj(t, slot):
            g = t // NB
            i = t % NB
            OC = 2 * LANES
            for b in range(BQ // OC):
                y = None
                for r in range(REP):
                    part = _nt(_bf(wou_v[g * REP + r]), _bf(ao_v[slot, r, b * (OC // 2):(b + 1) * (OC // 2), :]))
                    y = part if y is None else y + part
                for n in range(OC // LANES):
                    ti = i * (BQ // LANES) + b * (OC // LANES) + n
                    accT_v[ti] += y[:, n * LANES:(n + 1) * LANES]

        for cp in grp_copies(0, sem_g.at[0]):
            cp.wait()
        qproj(0, 0)

        def body(t, _):
            g = t // NB
            i = t % NB

            @pl.when((i == 0) & (g + 2 < HKV))
            def _():
                for cp in grp_copies(g + 2, sem_g.at[g % 2]):
                    cp.start()

            @pl.when(t == NB)
            def _():
                for cp in cp_moe:
                    cp.start()

            @pl.when((i == NB - 1) & (g + 1 < HKV))
            def _():
                for cp in grp_copies(g + 1, sem_g.at[(g + 1) % 2]):
                    cp.wait()

            slot = t % 2
            pcs = attn_pieces(t, slot, t // T)
            pcs['Q'] = lambda: qproj(jnp.minimum(t + 1, T - 1), 1 - slot)
            pcs['O'] = lambda: oproj(jnp.maximum(t - 1, 0), 1 - slot)
            for name in order:
                pcs[name]()
            return _

        lax.fori_loop(0, T, body, None)
        oproj(T - 1, (T - 1) % 2)

        cp_wm[1].wait()
        mod_b = _r(_mm(sc8, wm_v[:, 2 * D:6 * D]))[0:1]
        rows5 = [mod_b[:, 0:D], mod_b[:, D:2 * D], _r(1.0 + mod_b[:, 2 * D:3 * D]), mod_b[:, 3 * D:4 * D],
                 jnp.broadcast_to(wr_ref[...].astype(F32), (1, D))]
        GA, SB, CB1, GB, WR = range(5)
        for j in range(5):
            col_v[j] = jnp.transpose(jnp.broadcast_to(rows5[j], (LANES, D)))

        def ln2_tile(i):
            x1 = _r(xT_v[i].astype(F32) + col_v[GA] * accT_v[i])
            m = jnp.sum(x1, axis=0, keepdims=True) * (1.0 / D)
            xc = x1 - m
            var = jnp.sum(xc * xc, axis=0, keepdims=True) * (1.0 / D)
            inv = 1.0 / _r(jnp.sqrt(_r(_r(var) + _r(jnp.float32(EPS)))))
            h = _r(_r(_r(_r(x1 - _r(m)) * inv) * col_v[CB1]) + col_v[SB])
            accT_v[i] = x1
            h2T_v[i] = h.astype(BF16)
            r_v[pl.ds(i, 1), :] = jnp.sum(h * col_v[WR], axis=0, keepdims=True)

        def ln2_body(i, _):
            for u in range(lnu):
                ln2_tile(i * lnu + u)
            return _

        lax.fori_loop(0, NT // lnu, ln2_body, None)

        r = _r(r_v[...]) + 0.0
        r = jnp.where(r != r, -jnp.inf, r)
        pos = (lax.broadcasted_iota(jnp.int32, (NT, LANES), 0) * LANES
               + lax.broadcasted_iota(jnp.int32, (NT, LANES), 1))
        taken = jnp.zeros((NT, LANES), jnp.bool_)
        lane = lax.broadcasted_iota(jnp.int32, (8, S), 1)
        sub = lax.broadcasted_iota(jnp.int32, (8, S), 0)
        onehot = jnp.zeros((8, S), F32)
        subl = lax.broadcasted_iota(jnp.int32, (8, LANES), 0)
        rsel = jnp.zeros((8, LANES), F32)
        for j in range(TOPC):
            rm = jnp.where(taken, -jnp.inf, r)
            mx = jnp.max(rm)
            cand = jnp.where((rm == mx) & (~taken), pos, S)
            idx = jnp.min(cand.astype(F32)).astype(jnp.int32)
            taken = taken | (pos == idx)
            onehot = jnp.where((sub == j) & (lane == idx), 1.0, onehot)
            rsel = jnp.where(subl == j, mx, rsel)
        oh = onehot.astype(BF16)
        oh_v[...] = jnp.concatenate([oh, jnp.zeros((LANES - 8, S), BF16)], axis=0)

        xs = None
        for i in range(NT):
            part = _nt(oh[:, i * LANES:(i + 1) * LANES], h2T_v[i])
            xs = part if xs is None else xs + part
        xs = xs.astype(BF16)
        for cp in cp_moe:
            cp.wait()
        gt = _r(_mm(xs, wg_v[...]))
        gt = _r(gt * _r(jax.nn.sigmoid(gt)))
        ut = _r(_mm(xs, wu_v[...]))
        y = _r(_nt((gt * ut).astype(BF16), wdT_v[...]))
        y = _r(y * _r(jax.nn.sigmoid(rsel[:, 0:1])))
        gy = y * rows5[GB]
        yT = jnp.transpose(jnp.concatenate([gy, jnp.zeros((LANES - 8, D), F32)], axis=0)).astype(BF16)

        for i in range(NT):
            h = h2T_v[i].astype(F32)
            accT_v[i] = accT_v[i] + col_v[GB] * (h + h * 0.0)

        for ch in range(XCH):
            for i in range(ch * TPC, (ch + 1) * TPC):
                upd = _mm(yT, oh_v[:, i * LANES:(i + 1) * LANES])
                xT_v[i] = (accT_v[i] + upd).astype(BF16)
            for cp in o_copies(ch):
                cp.start()
        for ch in range(XCH):
            for cp in o_copies(ch):
                cp.wait()

    return kernel


def make(BQ=512, XCH=4, lnu=1, vmem_mb=127):
    @jax.jit
    def fn(A_x, A_k_cache, A_v_cache, A_wq, A_wo, B_x, B_w_r, B_w_gate, B_w_up, B_w_down, c, w_mod):
        del B_x
        B, S, D = A_x.shape
        _, HKV, SK, _ = A_k_cache.shape
        F = B_w_gate.shape[1]
        REP = HQ // HKV
        NT = S // LANES
        NBLK = REP * BQ // 128
        any_spec = pl.BlockSpec(memory_space=pl.ANY)
        vmem_spec = pl.BlockSpec(memory_space=pltpu.VMEM)
        out = pl.pallas_call(
            _make_kernel(S, D, HKV, SK, F, BQ, XCH, lnu),
            out_shape=jax.ShapeDtypeStruct((D, S), BF16),
            in_specs=[any_spec, any_spec, any_spec, any_spec, any_spec, vmem_spec,
                      any_spec, any_spec, any_spec, vmem_spec, any_spec],
            out_specs=any_spec,
            scratch_shapes=[
                pltpu.VMEM((NT, D, LANES), BF16),
                pltpu.VMEM((HKV, SK, DH), BF16),
                pltpu.VMEM((HKV, SK, DH), BF16),
                pltpu.VMEM((HQ, D, DH), BF16),
                pltpu.VMEM((HQ, D, DH), BF16),
                pltpu.VMEM((D, F), BF16),
                pltpu.VMEM((D, F), BF16),
                pltpu.VMEM((D, F), BF16),
                pltpu.VMEM((D, 6 * D), BF16),
                pltpu.VMEM((S // 2, D), U32),
                pltpu.VMEM((2, REP, BQ // 2, DH), U32),
                pltpu.VMEM((2, REP, BQ // 2, DH), U32),
                pltpu.VMEM((NT, D, LANES), F32),
                pltpu.VMEM((5, D, LANES), F32),
                pltpu.VMEM((NT, D, LANES), BF16),
                pltpu.VMEM((NT, LANES), F32),
                pltpu.VMEM((LANES, S), BF16),
                pltpu.SemaphoreType.DMA((XCH,)),
                pltpu.SemaphoreType.DMA((2,)),
                pltpu.SemaphoreType.DMA((2,)),
                pltpu.SemaphoreType.DMA(()),
                pltpu.SemaphoreType.DMA(()),
            ]
            + [pltpu.VMEM((1, 128, SK), F32)] * NBLK
            + [pltpu.VMEM((1, SK // LANES + 2, 64, LANES), U32)] * NBLK
            + [pltpu.VMEM((1, 128, LANES), F32)] * NBLK,
            compiler_params=pltpu.CompilerParams(vmem_limit_bytes=vmem_mb * 1024 * 1024),
        )(A_x.reshape(S, D).T, A_k_cache.reshape(HKV, SK, DH), A_v_cache.reshape(HKV, SK, DH),
          A_wq, A_wo.T, B_w_r.reshape(1, D), B_w_gate, B_w_up, B_w_down.T, c, w_mod)
        return out.T.reshape(B, S, D)

    return fn


pallas_adaLN_cond__gqa_block_cached__moe_arch_mod__prompt_kernel = make()
```

```python
import jax
import jax.numpy as jnp
from jax import lax
from jax.experimental import pallas as pl
from jax.experimental.pallas import tpu as pltpu

HQ, DH = 32, 128
TOPC = 8
EPS = 1e-5
LOG2E = 1.4426950408889634
LANES = 128

F32 = jnp.float32
BF16 = jnp.bfloat16
U32 = jnp.uint32


def _r(x):
    return x.astype(BF16).astype(F32)


def _r2(a, b):
    u = pltpu.pack_elementwise([a, b], packed_dtype=BF16)
    return tuple(pltpu.unpack_elementwise(u, index=i, packed_dtype=BF16, unpacked_dtype=F32) for i in range(2))


def _nt(a, b):
    return lax.dot_general(a, b, (((1,), (1,)), ((), ())), preferred_element_type=F32)


def _mm(a, b):
    return jnp.dot(a, b, preferred_element_type=F32)


def _pack(a, b):
    return pltpu.pack_elementwise([a, b], packed_dtype=BF16)


def _pack16(x):
    parts = [_pack(x[16 * i:16 * i + 8], x[16 * i + 8:16 * i + 16]) for i in range(x.shape[0] // 16)]
    return parts[0] if len(parts) == 1 else jnp.concatenate(parts, axis=0)


def _bf(x):
    return pltpu.bitcast(x, BF16)


def _recip(l):
    r = pl.reciprocal(l, approx=True)
    return r * (2.0 - l * r)


def _order(nblk, opos, qpos):
    o = []
    for j in range(nblk):
        o += [f'A{j}', f'B{j}'] + ([f'C{j-1}'] if j else [])
    o += [f'C{nblk-1}']
    o.insert(o.index(opos), 'O')
    if qpos == 'end':
        o.append('Q')
    else:
        o.insert(o.index(qpos), 'Q')
    return o


def _make_kernel(S, D, HKV, SK, F, BQ, UNR, LN2M, OPOS, QPOS):
    REP = HQ // HKV
    NB = S // BQ
    T = HKV * NB
    NT = S // LANES
    MQ = 128
    KR = 512
    NR = SK // KR
    NKT = SK // LANES
    DM = D // LANES * LANES
    blocks = [(r, b) for r in range(REP) for b in range(BQ // MQ)]
    NBLK = len(blocks)
    WA = 2 * D // LANES
    assert (2 * D) % LANES == 0
    IB = S.bit_length() - 1
    assert S == 1 << IB and IB <= 14
    XCH = NB
    TPC = NT // XCH

    def kernel(xT_hbm, k_hbm, v_hbm, wq_hbm, woT_hbm, wr_ref, wg_hbm, wu_hbm, wdT_hbm, c_ref, wm_hbm,
               oT_hbm,
               xT_v, k_v, v_v, wq_v, woT_v, wg_v, wu_v, wdT_v, wm_v,
               h_v, q_v, ao_v, accT_v, x1_v, col_v, gb_v, gt_v, h2T_v, r_v, oh_v,
               sem_x, sem_wm, sem_g0, sem_g, sem_moe, sem_o, sem_p, *sp):
        s_v = sp[:NBLK]
        p_v = sp[NBLK:2 * NBLK]
        m_v = sp[2 * NBLK:3 * NBLK]
        ku_v = k_v.bitcast(U32)
        vu_v = v_v.bitcast(U32)
        wqu_v = wq_v.bitcast(U32)
        wou_v = woT_v.bitcast(U32)

        def wq_copies(g, sem):
            return [pltpu.make_async_copy(wq_hbm.at[:, pl.ds(pl.multiple_of((g * REP + r) * DH, DH), DH)],
                                          wq_v.at[g * REP + r], sem) for r in range(REP)]

        def kv_copies(g, sem):
            return [pltpu.make_async_copy(k_hbm.at[g], k_v.at[g], sem),
                    pltpu.make_async_copy(v_hbm.at[g], v_v.at[g], sem)]

        def wo_copies(g, sem):
            return [pltpu.make_async_copy(woT_hbm.at[:, pl.ds(pl.multiple_of((g * REP + r) * DH, DH), DH)],
                                          woT_v.at[g * REP + r], sem) for r in range(REP)]

        def grp_copies(g, sem):
            return wq_copies(g, sem) + kv_copies(g, sem) + wo_copies(g, sem)

        def x_copies(ch):
            return [pltpu.make_async_copy(xT_hbm.at[:, pl.ds(i * LANES, LANES)], xT_v.at[i], sem_x.at[ch])
                    for i in range(ch * TPC, (ch + 1) * TPC)]

        def x_chunk_wait(ch):
            dst = xT_v.at[pl.ds(ch * TPC, TPC)]
            pltpu.make_async_copy(dst, dst, sem_x.at[ch]).wait()

        def o_copies(tiles):
            return [pltpu.make_async_copy(xT_v.at[i], oT_hbm.at[:, pl.ds(pl.multiple_of(i * LANES, LANES), LANES)], sem_o)
                    for i in tiles]

        cp_wm = (
            pltpu.make_async_copy(wm_hbm.at[:, pl.ds(0, 2 * D)], wm_v.at[:, pl.ds(0, 2 * D)], sem_wm.at[0]),
            pltpu.make_async_copy(wm_hbm.at[:, pl.ds(2 * D, 4 * D)], wm_v.at[:, pl.ds(2 * D, 4 * D)], sem_wm.at[1]),
        )
        cp_moe = (
            pltpu.make_async_copy(wg_hbm, wg_v, sem_moe),
            pltpu.make_async_copy(wu_hbm, wu_v, sem_moe),
            pltpu.make_async_copy(wdT_hbm, wdT_v, sem_moe),
        )

        cp_wm[0].start()
        for cp in x_copies(0):
            cp.start()

        def z_body(i, _):
            accT_v[i] = jnp.zeros((D, LANES), F32)
            return _
        lax.fori_loop(0, NT, z_body, None)
        ao_v[...] = jnp.zeros((REP, BQ // 2, DH), U32)

        cf = c_ref[...].astype(F32)
        sc = _r(cf * _r(jax.nn.sigmoid(cf))).astype(BF16)
        sc8 = jnp.broadcast_to(sc, (8, D))
        cp_wm[0].wait()
        for ch in range(1, XCH):
            for cp in x_copies(ch):
                cp.start()
        mod_a = _r(_mm(sc8, wm_v[:, 0:2 * D]))[0:1]
        sa = mod_a[:, 0:D]
        ca1 = _r(1.0 + mod_a[:, D:2 * D])

        eye = (lax.broadcasted_iota(jnp.int32, (LANES, LANES), 0)
               == lax.broadcasted_iota(jnp.int32, (LANES, LANES), 1)).astype(BF16)

        def ln1_block(b, zero):
            tiles = [b * TPC + u for u in range(TPC)]
            slabs = [slice(16 * c, 16 * c + 16) for c in range(D // 16)]
            tot = [None] * TPC
            for sl in slabs:
                for u, i in enumerate(tiles):
                    x = xT_v[i, sl, :].astype(F32)
                    tot[u] = x[0:8] + x[8:16] if tot[u] is None else tot[u] + (x[0:8] + x[8:16])
            mean = [jnp.sum(t_, axis=0, keepdims=True) * (1.0 / D) for t_ in tot]
            sq = [None] * TPC
            for sl in slabs:
                for u, i in enumerate(tiles):
                    xc = xT_v[i + zero, sl, :].astype(F32) - mean[u]
                    xx = xc * xc
                    sq[u] = xx[0:8] + xx[8:16] if sq[u] is None else sq[u] + (xx[0:8] + xx[8:16])
            inv = [lax.rsqrt(jnp.sum(t_, axis=0, keepdims=True) * (1.0 / D) + EPS) for t_ in sq]
            for u, i in enumerate(tiles):
                xh = ((xT_v[i + zero].astype(F32) - mean[u]) * inv[u]).astype(BF16)
                xn = _nt(eye, xh)
                h_v[pl.ds(pl.multiple_of(i * (LANES // 2), LANES // 2), LANES // 2), :] = \
                    _pack16(_r(xn * ca1) + sa)

        def ln1_body(b, z):
            x_chunk_wait(b)

            @pl.when(b == 1)
            def _():
                for cp in wq_copies(0, sem_g0.at[0]) + kv_copies(0, sem_g0.at[1]) + wo_copies(0, sem_g0.at[2]):
                    cp.start()

            ln1_block(b, z)
            return z + b // NB

        lax.fori_loop(0, NB, ln1_body, 0)

        qscale = LOG2E * DH ** -0.5

        def attn_pieces(g, slot, zero):

            def a_step(j):
                def f():
                    r, b = blocks[j]
                    q = _bf(q_v[r, b * (MQ // 2):(b + 1) * (MQ // 2), :])
                    mp = None
                    for rd in range(NR):
                        s = _nt(q, _bf(ku_v[g, rd * (KR // 2):(rd + 1) * (KR // 2), :]))
                        s_v[j][0, :, rd * KR:(rd + 1) * KR] = s
                        for n in range(KR // LANES):
                            sn = s[:, n * LANES:(n + 1) * LANES]
                            mp = sn if mp is None else jnp.maximum(mp, sn)
                    m_v[j][0] = jnp.broadcast_to(jnp.max(mp, axis=1, keepdims=True), (MQ, LANES))
                return f

            def b_step(j):
                def f():
                    chain = None
                    for c in range(MQ // 16):
                        ra = slice(c * 16, c * 16 + 8)
                        rb = slice(c * 16 + 8, c * 16 + 16)
                        ma = m_v[j][zero, ra, :]
                        mb = m_v[j][zero, rb, :]
                        if chain is not None:
                            ma = jnp.maximum(ma, jnp.minimum(chain[0], ma))
                            mb = jnp.maximum(mb, jnp.minimum(chain[1], mb))
                        la = lb = None
                        for n in range(NKT):
                            cols = slice(n * LANES, (n + 1) * LANES)
                            pa = jnp.exp2(s_v[j][zero, ra, cols] - ma)
                            pb = jnp.exp2(s_v[j][zero, rb, cols] - mb)
                            p_v[j][0, n, c * 8:c * 8 + 8, :] = _pack(pa, pb)
                            la = pa if la is None else la + pa
                            lb = pb if lb is None else lb + pb
                        chain = (la, lb)
                        base = 16 * (c % 4)
                        lp = NKT + c // 4
                        p_v[j][0, lp, pl.ds(base, 8, stride=2), :] = pltpu.bitcast(
                            jnp.broadcast_to(jnp.sum(la, axis=1, keepdims=True), (8, LANES)), U32)
                        p_v[j][0, lp, pl.ds(base + 1, 8, stride=2), :] = pltpu.bitcast(
                            jnp.broadcast_to(jnp.sum(lb, axis=1, keepdims=True), (8, LANES)), U32)
                return f

            def c_step(j):
                def f():
                    r, b = blocks[j]
                    o = None
                    for rd in range(NR):
                        pp = _bf(jnp.concatenate(
                            [p_v[j][zero, rd * (KR // LANES) + n] for n in range(KR // LANES)], axis=1))
                        part = _mm(pp, _bf(vu_v[g, rd * (KR // 2):(rd + 1) * (KR // 2), :]))
                        o = part if o is None else o + part
                    l = jnp.concatenate([pltpu.bitcast(p_v[j][zero, NKT + c], F32) for c in range(2)], axis=0)
                    ao_v[r, b * (MQ // 2):(b + 1) * (MQ // 2), :] = _pack16(o * _recip(l))
                return f

            pieces = {}
            for j in range(NBLK):
                pieces[f'A{j}'] = a_step(j)
                pieces[f'B{j}'] = b_step(j)
                pieces[f'C{j}'] = c_step(j)
            return pieces

        def qproj(g, i, slot):
            rows = pl.ds(pl.multiple_of(i * (BQ // 2), BQ // 2), BQ // 2)
            hm = _bf(h_v[rows, 0:DM])
            mains = [_mm(hm, _bf(wqu_v[g * REP + r, 0:DM // 2, :])) for r in range(REP)]
            for r in range(REP):
                wt = _bf(wqu_v[g * REP + r, DM // 2:D // 2, :])
                for b in range(BQ // MQ):
                    rws = pl.ds(pl.multiple_of(i * (BQ // 2) + b * (MQ // 2), MQ // 2), MQ // 2)
                    qq = mains[r][b * MQ:(b + 1) * MQ] + _mm(_bf(h_v[rws, DM:D]), wt)
                    q_v[r, b * (MQ // 2):(b + 1) * (MQ // 2), :] = _pack16(qq * qscale)

        def oproj(g, i, slot):
            OC = 2 * LANES
            for b in range(BQ // OC):
                y = None
                for r in range(REP):
                    part = _nt(_bf(wou_v[g * REP + r]), _bf(ao_v[r, b * (OC // 2):(b + 1) * (OC // 2), :]))
                    y = part if y is None else y + part
                for n in range(OC // LANES):
                    ti = i * (BQ // LANES) + b * (OC // LANES) + n
                    accT_v[ti] += y[:, n * LANES:(n + 1) * LANES]

        for cp in wq_copies(0, sem_g0.at[0]):
            cp.wait()
        qproj(0, 0, 0)
        for cp in kv_copies(0, sem_g0.at[1]) + wo_copies(0, sem_g0.at[2]):
            cp.wait()
        for cp in grp_copies(1, sem_g.at[1]):
            cp.start()
        cp_wm[1].start()

        GA, SB, CB1, GB = range(4)
        wr8 = jnp.broadcast_to(wr_ref[...].reshape(1, D), (8, D))

        def mod_columns():
            cp_wm[1].wait()
            mod_b = _r(_mm(sc8, wm_v[:, 2 * D:6 * D]))[0:1]
            rows5 = [mod_b[:, 0:D], mod_b[:, D:2 * D], _r(1.0 + mod_b[:, 2 * D:3 * D]), mod_b[:, 3 * D:4 * D]]
            for j in range(4):
                col_v[j] = jnp.transpose(jnp.broadcast_to(rows5[j], (LANES, D)))
            gb_v[...] = jnp.broadcast_to(rows5[GB], (8, D))

        def ln2_block(b, zero):
            tiles = [b * TPC + u for u in range(TPC)]
            slabs = [(slice(16 * c, 16 * c + 8), slice(16 * c + 8, 16 * c + 16)) for c in range(D // 16)]
            tot = [None] * TPC
            for sa_, sb_ in slabs:
                sl = slice(sa_.start, sb_.stop)
                ga = col_v[GA, sl, :]
                for u, ti in enumerate(tiles):
                    t_ = xT_v[ti, sl, :].astype(F32) + ga * accT_v[ti, sl, :]
                    x1a, x1b = _r2(t_[0:8], t_[8:16])
                    x1_v[ti, sa_, :] = x1a
                    x1_v[ti, sb_, :] = x1b
                    tot[u] = x1a + x1b if tot[u] is None else tot[u] + (x1a + x1b)
            mean = [jnp.sum(t_, axis=0, keepdims=True) * (1.0 / D) for t_ in tot]
            sq = [None] * TPC
            for sa_, sb_ in slabs:
                for u, ti in enumerate(tiles):
                    xa = x1_v[ti + zero, sa_, :] - mean[u]
                    xb = x1_v[ti + zero, sb_, :] - mean[u]
                    xx = xa * xa + xb * xb
                    sq[u] = xx if sq[u] is None else sq[u] + xx
            var = [jnp.sum(t_, axis=0, keepdims=True) * (1.0 / D) for t_ in sq]
            inv = [1.0 / _r(jnp.sqrt(_r(_r(v_) + _r(jnp.float32(EPS))))) for v_ in var]
            mb = [_r(m_) for m_ in mean]
            for sa_, sb_ in slabs:
                sl = slice(sa_.start, sb_.stop)
                cb1, sb, gb = col_v[CB1, sl, :], col_v[SB, sl, :], col_v[GB, sl, :]
                for u, ti in enumerate(tiles):
                    a_, b_ = _r2(x1_v[ti + zero, sa_, :] - mb[u], x1_v[ti + zero, sb_, :] - mb[u])
                    a_, b_ = _r2(a_ * inv[u], b_ * inv[u])
                    a_, b_ = _r2(a_ * cb1[0:8], b_ * cb1[8:16])
                    hb = (jnp.concatenate([a_, b_], axis=0) + sb).astype(BF16)
                    h2T_v[ti, sl, :] = hb
                    h = hb.astype(F32)
                    base = x1_v[ti + zero, sl, :] + gb * (h + h * 0.0)
                    accT_v[ti, sl, :] = base
                    xT_v[ti, sl, :] = base.astype(BF16)
            for ti in tiles:
                r_v[pl.ds(ti, 1), :] = _mm(wr8, h2T_v[ti + zero])[0:1, :]
            for cp in o_copies(tiles):
                cp.start()

        def step(g, i, extra):
            t = g * NB + i
            slot = i % 2
            tn = jnp.minimum(t + 1, T - 1)
            tp = jnp.maximum(t - 1, 0)
            pcs = attn_pieces(g, slot, t // T)
            pcs['Q'] = lambda: qproj(tn // NB, tn % NB, 1 - slot)
            pcs['O'] = lambda: oproj(tp // NB, tp % NB, 1 - slot)

            order = _order(NBLK, OPOS, QPOS)
            for name in order:
                pcs[name]()

        def group_body(g, _):
            @pl.when(g + 2 < HKV)
            def _():
                for cp in grp_copies(g + 2, sem_g.at[g % 2]):
                    cp.start()
            @pl.when(g == 1)
            def _():
                for cp in cp_moe:
                    cp.start()

            @pl.when(g + 1 < HKV)
            def _():
                for cp in grp_copies(g + 1, sem_g.at[(g + 1) % 2]):
                    cp.wait()

            def inner(i, _):
                step(g, i, None)
                return _
            lax.fori_loop(0, NB, inner, None, unroll=UNR)
            return _

        def group_body_z(g, z):
            group_body(g, None)
            return z + g // HKV

        zero_t = lax.fori_loop(0, HKV, group_body_z, 0)
        mod_columns()
        oproj(HKV - 1, NB - 1, 0)
        if LN2M == 0:
            for b in range(NB):
                ln2_block(b, zero_t)
        elif LN2M == 1:
            lax.fori_loop(0, NB, lambda b, c_: (ln2_block(b, zero_t), c_)[1], 0)
        else:
            ln2_block(0, zero_t)
            lax.fori_loop(1, NB, lambda b, c_: (ln2_block(b, zero_t), c_)[1], 0)

        r = _r(r_v[...]) + 0.0
        r = jnp.where(r != r, -jnp.inf, r)
        pos = (lax.broadcasted_iota(jnp.int32, (NT, LANES), 0) * LANES
               + lax.broadcasted_iota(jnp.int32, (NT, LANES), 1))
        b16 = lax.shift_right_logical(pltpu.bitcast(r, jnp.int32), 16)
        s16 = jnp.where(b16 >= 0x8000, 0xFFFF - b16, b16 + 0x8000)
        key0 = pltpu.bitcast((s16 * S + (S - 1 - pos)) + 0x10000000, F32)
        key = key0
        subl = lax.broadcasted_iota(jnp.int32, (8, LANES), 0)
        sel = jnp.zeros((8, LANES), F32)
        for j in range(TOPC):
            mx = jnp.max(jnp.max(key, axis=0, keepdims=True), axis=1, keepdims=True)
            key = jnp.where(key == mx, 0.0, key)
            sel = jnp.where(subl == j, mx, sel)
        bits = pltpu.bitcast(sel, jnp.int32) - 0x10000000
        tile_v = lax.shift_right_logical((S - 1) - (bits & (S - 1)), 7)
        tile_s = [tile_v[j, 0] for j in range(TOPC)]
        for i in range(NT):
            oh_v[i] = jnp.concatenate([(key0[i:i + 1, :] == sel).astype(BF16),
                                       jnp.zeros((LANES - 8, LANES), BF16)], axis=0)
        ssel = lax.shift_right_logical(bits, IB)
        bsel = jnp.where(ssel >= 0x8000, ssel - 0x8000, 0xFFFF - ssel)
        rsel = pltpu.bitcast(lax.shift_left(bsel, 16), F32)

        xs = None
        for j in range(TOPC):
            row = jnp.where(subl == j, oh_v[tile_s[j], 0:8, :].astype(F32), 0.0).astype(BF16)
            part = _nt(row, h2T_v[tile_s[j]])
            xs = part if xs is None else xs + part
        xs = xs.astype(BF16)

        for cp in cp_moe:
            cp.wait()
        gt = _r(_mm(xs, wg_v[...]))
        gt = _r(gt * _r(jax.nn.sigmoid(gt)))
        ut = _r(_mm(xs, wu_v[...]))
        y = _r(_nt((gt * ut).astype(BF16), wdT_v[...]))
        y = _r(y * _r(jax.nn.sigmoid(rsel[:, 0:1])))
        gy = y * gb_v[...]
        yT = jnp.transpose(jnp.concatenate([gy, jnp.zeros((LANES - 8, D), F32)], axis=0)).astype(BF16)

        for cp in o_copies(range(NT)):
            cp.wait()
        RQ = D // 4 // 16 * 16

        def patch_copy(j):
            c0 = pl.multiple_of(tile_s[j] * LANES, LANES)
            return pltpu.make_async_copy(h2T_v.at[j], oT_hbm.at[:, pl.ds(c0, LANES)], sem_p.at[j])

        def first_use(j):
            ok = tile_s[j] >= 0
            for k in range(j):
                ok = ok & (tile_s[j] != tile_s[k])
            return ok

        for j in range(TOPC):
            oh = oh_v[tile_s[j]]
            for q4 in range(4):
                rows = slice(q4 * RQ, D if q4 == 3 else (q4 + 1) * RQ)
                h2T_v[j, rows, :] = (accT_v[tile_s[j], rows, :] + _mm(yT[rows], oh)).astype(BF16)
            pl.when(first_use(j))(lambda j=j: patch_copy(j).start())
        for j in range(TOPC):
            pl.when(first_use(j))(lambda j=j: patch_copy(j).wait())

    return kernel


def make(BQ=512, UNR=2, LN2M=2, OPOS='A1', QPOS='C6', vmem_mb=127):
    @jax.jit
    def fn(A_x, A_k_cache, A_v_cache, A_wq, A_wo, B_x, B_w_r, B_w_gate, B_w_up, B_w_down, c, w_mod):
        del B_x
        B, S, D = A_x.shape
        _, HKV, SK, _ = A_k_cache.shape
        F = B_w_gate.shape[1]
        REP = HQ // HKV
        NT = S // LANES
        NBLK = REP * BQ // 128
        any_spec = pl.BlockSpec(memory_space=pl.ANY)
        vmem_spec = pl.BlockSpec(memory_space=pltpu.VMEM)
        out = pl.pallas_call(
            _make_kernel(S, D, HKV, SK, F, BQ, UNR, LN2M, OPOS, QPOS),
            out_shape=jax.ShapeDtypeStruct((D, S), BF16),
            in_specs=[any_spec, any_spec, any_spec, any_spec, any_spec, vmem_spec,
                      any_spec, any_spec, any_spec, vmem_spec, any_spec],
            out_specs=any_spec,
            scratch_shapes=[
                pltpu.VMEM((NT, D, LANES), BF16),
                pltpu.VMEM((HKV, SK, DH), BF16),
                pltpu.VMEM((HKV, SK, DH), BF16),
                pltpu.VMEM((HQ, D, DH), BF16),
                pltpu.VMEM((HQ, D, DH), BF16),
                pltpu.VMEM((D, F), BF16),
                pltpu.VMEM((D, F), BF16),
                pltpu.VMEM((D, F), BF16),
                pltpu.VMEM((D, 6 * D), BF16),
                pltpu.VMEM((S // 2, D), U32),
                pltpu.VMEM((REP, BQ // 2, DH), U32),
                pltpu.VMEM((REP, BQ // 2, DH), U32),
                pltpu.VMEM((NT, D, LANES), F32),
                pltpu.VMEM((NT, D, LANES), F32),
                pltpu.VMEM((4, D, LANES), F32),
                pltpu.VMEM((8, D), F32),
                pltpu.VMEM((8, F), F32),
                pltpu.VMEM((NT, D, LANES), BF16),
                pltpu.VMEM((NT, LANES), F32),
                pltpu.VMEM((NT, LANES, LANES), BF16),
                pltpu.SemaphoreType.DMA((S // BQ,)),
                pltpu.SemaphoreType.DMA((2,)),
                pltpu.SemaphoreType.DMA((3,)),
                pltpu.SemaphoreType.DMA((2,)),
                pltpu.SemaphoreType.DMA(()),
                pltpu.SemaphoreType.DMA(()),
                pltpu.SemaphoreType.DMA((TOPC,)),
            ]
            + [pltpu.VMEM((1, 128, SK), F32)] * NBLK
            + [pltpu.VMEM((1, SK // LANES + 2, 64, LANES), U32)] * NBLK
            + [pltpu.VMEM((1, 128, LANES), F32)] * NBLK,
            compiler_params=pltpu.CompilerParams(vmem_limit_bytes=vmem_mb * 1024 * 1024),
        )(A_x.reshape(S, D).T, A_k_cache.reshape(HKV, SK, DH), A_v_cache.reshape(HKV, SK, DH),
          A_wq, A_wo.T, B_w_r, B_w_gate, B_w_up, B_w_down.T, c, w_mod)
        return out.T.reshape(B, S, D)

    return fn


pallas_adaLN_cond__gqa_block_cached__moe_arch_mod__prompt_kernel = make()
```

```python
import jax
import jax.numpy as jnp
from jax import lax
from jax.experimental import pallas as pl
from jax.experimental.pallas import tpu as pltpu

HQ, DH = 32, 128
TOPC = 8
EPS = 1e-5
LOG2E = 1.4426950408889634
LANES = 128

F32 = jnp.float32
BF16 = jnp.bfloat16
U32 = jnp.uint32


def _r(x):
    return x.astype(BF16).astype(F32)


def _r2(a, b):
    u = pltpu.pack_elementwise([a, b], packed_dtype=BF16)
    return tuple(pltpu.unpack_elementwise(u, index=i, packed_dtype=BF16, unpacked_dtype=F32) for i in range(2))


def _after(val, ref, zero):
    z = jnp.bitwise_and(pltpu.bitcast(ref, jnp.int32), zero)
    return pltpu.bitcast(jnp.bitwise_or(pltpu.bitcast(val, jnp.int32), z), F32)


def _nt(a, b):
    return lax.dot_general(a, b, (((1,), (1,)), ((), ())), preferred_element_type=F32)


def _mm(a, b):
    return jnp.dot(a, b, preferred_element_type=F32)


def _pack(a, b):
    return pltpu.pack_elementwise([a, b], packed_dtype=BF16)


def _pack16(x):
    parts = [_pack(x[16 * i:16 * i + 8], x[16 * i + 8:16 * i + 16]) for i in range(x.shape[0] // 16)]
    return parts[0] if len(parts) == 1 else jnp.concatenate(parts, axis=0)


def _bf(x):
    return pltpu.bitcast(x, BF16)


def _recip(l):
    r = pl.reciprocal(l, approx=True)
    return r * (2.0 - l * r)


def _order(nblk, opos, qpos):
    o = []
    for j in range(nblk):
        o += [f'A{j}', f'B{j}'] + ([f'C{j-1}'] if j else [])
    o += [f'C{nblk-1}']
    o.insert(o.index(opos), 'O')
    if qpos == 'end':
        o.append('Q')
    else:
        o.insert(o.index(qpos), 'Q')
    return o


def _make_kernel(S, D, HKV, SK, F, BQ, UNR, OPOS, QPOS):
    REP = HQ // HKV
    NB = S // BQ
    T = HKV * NB
    NT = S // LANES
    MQ = 128
    KR = 512
    NR = SK // KR
    NKT = SK // LANES
    DM = D // LANES * LANES
    blocks = [(r, b) for r in range(REP) for b in range(BQ // MQ)]
    NBLK = len(blocks)
    WA = 2 * D // LANES
    assert (2 * D) % LANES == 0
    IB = S.bit_length() - 1
    assert S == 1 << IB and IB <= 14
    XCH = NB
    TPC = NT // XCH

    def kernel(xT_hbm, k_hbm, v_hbm, wq_hbm, woT_hbm, wr_ref, wg_hbm, wu_hbm, wdT_hbm, c_ref, wm_hbm,
               oT_hbm,
               xT_v, k_v, v_v, wq_v, woT_v, wg_v, wu_v, wdT_v, wm_v,
               h_v, q_v, ao_v, accT_v, x1_v, col_v, gb_v, h2T_v, r_v, oh_v,
               sem_x, sem_wm, sem_g0, sem_g, sem_moe, sem_o, sem_p, *sp):
        s_v = sp[:NBLK]
        p_v = sp[NBLK:2 * NBLK]
        m_v = sp[2 * NBLK:3 * NBLK]
        ku_v = k_v.bitcast(U32)
        vu_v = v_v.bitcast(U32)
        wqu_v = wq_v.bitcast(U32)
        wou_v = woT_v.bitcast(U32)

        def wq_copies(g, sem):
            return [pltpu.make_async_copy(wq_hbm.at[:, pl.ds(pl.multiple_of((g * REP + r) * DH, DH), DH)],
                                          wq_v.at[g * REP + r], sem) for r in range(REP)]

        def kv_copies(g, sem):
            return [pltpu.make_async_copy(k_hbm.at[g], k_v.at[g], sem),
                    pltpu.make_async_copy(v_hbm.at[g], v_v.at[g], sem)]

        def wo_copies(g, sem):
            return [pltpu.make_async_copy(woT_hbm.at[:, pl.ds(pl.multiple_of((g * REP + r) * DH, DH), DH)],
                                          woT_v.at[g * REP + r], sem) for r in range(REP)]

        def grp_copies(g, sem):
            return wq_copies(g, sem) + kv_copies(g, sem) + wo_copies(g, sem)

        def x_copies(ch):
            return [pltpu.make_async_copy(xT_hbm.at[:, pl.ds(i * LANES, LANES)], xT_v.at[i], sem_x.at[ch])
                    for i in range(ch * TPC, (ch + 1) * TPC)]

        def x_chunk_wait(ch):
            dst = xT_v.at[pl.ds(ch * TPC, TPC)]
            pltpu.make_async_copy(dst, dst, sem_x.at[ch]).wait()

        def o_copies(tiles):
            return [pltpu.make_async_copy(xT_v.at[i], oT_hbm.at[:, pl.ds(pl.multiple_of(i * LANES, LANES), LANES)], sem_o)
                    for i in tiles]

        cp_wm = (
            pltpu.make_async_copy(wm_hbm.at[:, pl.ds(0, 2 * D)], wm_v.at[:, pl.ds(0, 2 * D)], sem_wm.at[0]),
            pltpu.make_async_copy(wm_hbm.at[:, pl.ds(2 * D, 4 * D)], wm_v.at[:, pl.ds(2 * D, 4 * D)], sem_wm.at[1]),
        )
        cp_moe = (
            pltpu.make_async_copy(wg_hbm, wg_v, sem_moe),
            pltpu.make_async_copy(wu_hbm, wu_v, sem_moe),
            pltpu.make_async_copy(wdT_hbm, wdT_v, sem_moe),
        )

        cp_wm[0].start()
        for cp in x_copies(0):
            cp.start()

        def z_body(i, _):
            accT_v[i] = jnp.zeros((D, LANES), F32)
            return _
        lax.fori_loop(0, NT, z_body, None)
        ao_v[...] = jnp.zeros((REP, BQ // 2, DH), U32)

        cf = c_ref[...].astype(F32)
        sc = _r(cf * _r(jax.nn.sigmoid(cf))).astype(BF16)
        sc8 = jnp.broadcast_to(sc, (8, D))
        cp_wm[0].wait()
        for ch in range(1, XCH):
            for cp in x_copies(ch):
                cp.start()
        mod_a = _r(_mm(sc8, wm_v[:, 0:2 * D]))[0:1]
        sa = mod_a[:, 0:D]
        ca1 = _r(1.0 + mod_a[:, D:2 * D])

        eye = (lax.broadcasted_iota(jnp.int32, (LANES, LANES), 0)
               == lax.broadcasted_iota(jnp.int32, (LANES, LANES), 1)).astype(BF16)

        def ln1_block(b, zero):
            tiles = [b * TPC + u for u in range(TPC)]
            slabs = [slice(16 * c, 16 * c + 16) for c in range(D // 16)]
            tot = [None] * TPC
            for sl in slabs:
                for u, i in enumerate(tiles):
                    x = xT_v[i, sl, :].astype(F32)
                    tot[u] = x[0:8] + x[8:16] if tot[u] is None else tot[u] + (x[0:8] + x[8:16])
            mean = [jnp.sum(t_, axis=0, keepdims=True) * (1.0 / D) for t_ in tot]
            sq = [None] * TPC
            for sl in slabs:
                for u, i in enumerate(tiles):
                    xc = xT_v[i + zero, sl, :].astype(F32) - mean[u]
                    xx = xc * xc
                    sq[u] = xx[0:8] + xx[8:16] if sq[u] is None else sq[u] + (xx[0:8] + xx[8:16])
            inv = [lax.rsqrt(jnp.sum(t_, axis=0, keepdims=True) * (1.0 / D) + EPS) for t_ in sq]
            for u, i in enumerate(tiles):
                xh = ((xT_v[i + zero].astype(F32) - mean[u]) * inv[u]).astype(BF16)
                xn = _nt(eye, xh)
                h_v[pl.ds(pl.multiple_of(i * (LANES // 2), LANES // 2), LANES // 2), :] = \
                    _pack16(_r(xn * ca1) + sa)

        def ln1_body(b, z):
            x_chunk_wait(b)

            @pl.when(b == 1)
            def _():
                for cp in wq_copies(0, sem_g0.at[0]) + kv_copies(0, sem_g0.at[1]) + wo_copies(0, sem_g0.at[2]):
                    cp.start()

            ln1_block(b, z)
            return z + b // NB

        lax.fori_loop(0, NB, ln1_body, 0)

        qscale = LOG2E * DH ** -0.5

        def attn_pieces(g, slot, zero):

            def a_step(j):
                def f():
                    r, b = blocks[j]
                    q = _bf(q_v[r, b * (MQ // 2):(b + 1) * (MQ // 2), :])
                    mp = None
                    for rd in range(NR):
                        s = _nt(q, _bf(ku_v[g, rd * (KR // 2):(rd + 1) * (KR // 2), :]))
                        s_v[j][0, :, rd * KR:(rd + 1) * KR] = s
                        for n in range(KR // LANES):
                            sn = s[:, n * LANES:(n + 1) * LANES]
                            mp = sn if mp is None else jnp.maximum(mp, sn)
                    m_v[j][0] = jnp.broadcast_to(jnp.max(mp, axis=1, keepdims=True), (MQ, LANES))
                return f

            def b_step(j):
                def f():
                    chain = None
                    for c in range(MQ // 16):
                        ra = slice(c * 16, c * 16 + 8)
                        rb = slice(c * 16 + 8, c * 16 + 16)
                        ma = m_v[j][zero, ra, :]
                        mb = m_v[j][zero, rb, :]
                        if chain is not None:
                            ma = _after(ma, chain[0], zero)
                            mb = _after(mb, chain[1], zero)
                        la = lb = None
                        for n in range(NKT):
                            cols = slice(n * LANES, (n + 1) * LANES)
                            pa = jnp.exp2(s_v[j][zero, ra, cols] - ma)
                            pb = jnp.exp2(s_v[j][zero, rb, cols] - mb)
                            p_v[j][0, n, c * 8:c * 8 + 8, :] = _pack(pa, pb)
                            la = pa if la is None else la + pa
                            lb = pb if lb is None else lb + pb
                        chain = (la, lb)
                        base = 16 * (c % 4)
                        lp = NKT + c // 4
                        p_v[j][0, lp, pl.ds(base, 8, stride=2), :] = pltpu.bitcast(
                            jnp.broadcast_to(jnp.sum(la, axis=1, keepdims=True), (8, LANES)), U32)
                        p_v[j][0, lp, pl.ds(base + 1, 8, stride=2), :] = pltpu.bitcast(
                            jnp.broadcast_to(jnp.sum(lb, axis=1, keepdims=True), (8, LANES)), U32)
                return f

            def c_step(j):
                def f():
                    r, b = blocks[j]
                    o = None
                    for rd in range(NR):
                        pp = _bf(jnp.concatenate(
                            [p_v[j][zero, rd * (KR // LANES) + n] for n in range(KR // LANES)], axis=1))
                        part = _mm(pp, _bf(vu_v[g, rd * (KR // 2):(rd + 1) * (KR // 2), :]))
                        o = part if o is None else o + part
                    l = jnp.concatenate([pltpu.bitcast(p_v[j][zero, NKT + c], F32) for c in range(2)], axis=0)
                    ao_v[r, b * (MQ // 2):(b + 1) * (MQ // 2), :] = _pack16(o * _recip(l))
                return f

            pieces = {}
            for j in range(NBLK):
                pieces[f'A{j}'] = a_step(j)
                pieces[f'B{j}'] = b_step(j)
                pieces[f'C{j}'] = c_step(j)
            return pieces

        def qproj(g, i, slot):
            rows = pl.ds(pl.multiple_of(i * (BQ // 2), BQ // 2), BQ // 2)
            hm = _bf(h_v[rows, 0:DM])
            mains = [_mm(hm, _bf(wqu_v[g * REP + r, 0:DM // 2, :])) for r in range(REP)]
            for r in range(REP):
                wt = _bf(wqu_v[g * REP + r, DM // 2:D // 2, :])
                for b in range(BQ // MQ):
                    rws = pl.ds(pl.multiple_of(i * (BQ // 2) + b * (MQ // 2), MQ // 2), MQ // 2)
                    tl = _mm(_bf(h_v[rws, DM:D]), wt)
                    qq = mains[r][b * MQ:(b + 1) * MQ] + tl
                    q_v[r, b * (MQ // 2):(b + 1) * (MQ // 2), :] = _pack16(qq * qscale)

        def oproj(g, i, slot):
            OC = 2 * LANES
            for b in range(BQ // OC):
                y = None
                for r in range(REP):
                    part = _nt(_bf(wou_v[g * REP + r]), _bf(ao_v[r, b * (OC // 2):(b + 1) * (OC // 2), :]))
                    y = part if y is None else y + part
                for n in range(OC // LANES):
                    ti = i * (BQ // LANES) + b * (OC // LANES) + n
                    accT_v[ti] += y[:, n * LANES:(n + 1) * LANES]

        for cp in wq_copies(0, sem_g0.at[0]):
            cp.wait()
        qproj(0, 0, 0)
        for cp in kv_copies(0, sem_g0.at[1]) + wo_copies(0, sem_g0.at[2]):
            cp.wait()
        for cp in grp_copies(1, sem_g.at[1]):
            cp.start()
        cp_wm[1].start()

        GA, SB, CB1, GB = range(4)
        wr8 = jnp.broadcast_to(wr_ref[...].reshape(1, D), (8, D))

        def mod_columns():
            cp_wm[1].wait()
            mod_b = _r(_mm(sc8, wm_v[:, 2 * D:6 * D]))[0:1]
            rows5 = [mod_b[:, 0:D], mod_b[:, D:2 * D], _r(1.0 + mod_b[:, 2 * D:3 * D]), mod_b[:, 3 * D:4 * D]]
            for j in range(4):
                col_v[j] = jnp.transpose(jnp.broadcast_to(rows5[j], (LANES, D)))
            gb_v[...] = jnp.broadcast_to(rows5[GB], (8, D))

        def ln2_block(b, zero):
            tiles = [b * TPC + u for u in range(TPC)]
            slabs = [(slice(16 * c, 16 * c + 8), slice(16 * c + 8, 16 * c + 16)) for c in range(D // 16)]
            tot = [None] * TPC
            for sa_, sb_ in slabs:
                sl = slice(sa_.start, sb_.stop)
                ga = col_v[GA, sl, :]
                for u, ti in enumerate(tiles):
                    t_ = xT_v[ti, sl, :].astype(F32) + ga * accT_v[ti, sl, :]
                    x1a, x1b = _r2(t_[0:8], t_[8:16])
                    x1_v[ti, sa_, :] = x1a
                    x1_v[ti, sb_, :] = x1b
                    tot[u] = x1a + x1b if tot[u] is None else tot[u] + (x1a + x1b)
            mean = [jnp.sum(t_, axis=0, keepdims=True) * (1.0 / D) for t_ in tot]
            sq = [None] * TPC
            for sa_, sb_ in slabs:
                for u, ti in enumerate(tiles):
                    xa = x1_v[ti + zero, sa_, :] - mean[u]
                    xb = x1_v[ti + zero, sb_, :] - mean[u]
                    xx = xa * xa + xb * xb
                    sq[u] = xx if sq[u] is None else sq[u] + xx
            var = [jnp.sum(t_, axis=0, keepdims=True) * (1.0 / D) for t_ in sq]
            inv = [1.0 / _r(jnp.sqrt(_r(_r(v_) + _r(jnp.float32(EPS))))) for v_ in var]
            mb = [_r(m_) for m_ in mean]
            for sa_, sb_ in slabs:
                sl = slice(sa_.start, sb_.stop)
                cb1, sb, gb = col_v[CB1, sl, :], col_v[SB, sl, :], col_v[GB, sl, :]
                for u, ti in enumerate(tiles):
                    a_, b_ = _r2(x1_v[ti + zero, sa_, :] - mb[u], x1_v[ti + zero, sb_, :] - mb[u])
                    a_, b_ = _r2(a_ * inv[u], b_ * inv[u])
                    a_, b_ = _r2(a_ * cb1[0:8], b_ * cb1[8:16])
                    hb = (jnp.concatenate([a_, b_], axis=0) + sb).astype(BF16)
                    h2T_v[ti, sl, :] = hb
                    h = hb.astype(F32)
                    base = x1_v[ti + zero, sl, :] + gb * (h + h * 0.0)
                    accT_v[ti, sl, :] = base
                    xT_v[ti, sl, :] = base.astype(BF16)
            for ti in tiles:
                r_v[pl.ds(ti, 1), :] = _mm(wr8, h2T_v[ti + zero])[0:1, :]
            for cp in o_copies(tiles):
                cp.start()

        def step(g, i, extra):
            t = g * NB + i
            slot = i % 2
            tn = jnp.minimum(t + 1, T - 1)
            tp = jnp.maximum(t - 1, 0)
            pcs = attn_pieces(g, slot, t // T)
            pcs['Q'] = lambda: qproj(tn // NB, tn % NB, 1 - slot)
            pcs['O'] = lambda: oproj(tp // NB, tp % NB, 1 - slot)

            order = _order(NBLK, OPOS, QPOS)
            for name in order:
                pcs[name]()

        def group_body(g, _):
            @pl.when(g + 2 < HKV)
            def _():
                for cp in grp_copies(g + 2, sem_g.at[g % 2]):
                    cp.start()
            @pl.when(g == 1)
            def _():
                for cp in cp_moe:
                    cp.start()

            @pl.when(g + 1 < HKV)
            def _():
                for cp in grp_copies(g + 1, sem_g.at[(g + 1) % 2]):
                    cp.wait()

            def inner(i, _):
                step(g, i, None)
                return _
            lax.fori_loop(0, NB, inner, None, unroll=UNR)
            return _

        def group_body_z(g, z):
            group_body(g, None)
            return z + g // HKV

        zero_t = lax.fori_loop(0, HKV, group_body_z, 0)
        mod_columns()
        oproj(HKV - 1, NB - 1, 0)
        ln2_block(0, zero_t)
        lax.fori_loop(1, NB, lambda b, c_: (ln2_block(b, zero_t), c_)[1], 0)

        r = _r(r_v[...]) + 0.0
        r = jnp.where(r != r, -jnp.inf, r)
        pos = (lax.broadcasted_iota(jnp.int32, (NT, LANES), 0) * LANES
               + lax.broadcasted_iota(jnp.int32, (NT, LANES), 1))
        b16 = lax.shift_right_logical(pltpu.bitcast(r, jnp.int32), 16)
        s16 = jnp.where(b16 >= 0x8000, 0xFFFF - b16, b16 + 0x8000)
        key0 = pltpu.bitcast((s16 * S + (S - 1 - pos)) + 0x10000000, F32)
        key = key0
        subl = lax.broadcasted_iota(jnp.int32, (8, LANES), 0)
        sel = jnp.zeros((8, LANES), F32)
        for j in range(TOPC):
            mx = jnp.max(jnp.max(key, axis=0, keepdims=True), axis=1, keepdims=True)
            key = jnp.where(key == mx, 0.0, key)
            sel = jnp.where(subl == j, mx, sel)
        bits = pltpu.bitcast(sel, jnp.int32) - 0x10000000
        tile_v = lax.shift_right_logical((S - 1) - (bits & (S - 1)), 7)
        tile_s = [tile_v[j, 0] for j in range(TOPC)]
        for i in range(NT):
            oh_v[i] = jnp.concatenate([(key0[i:i + 1, :] == sel).astype(BF16),
                                       jnp.zeros((LANES - 8, LANES), BF16)], axis=0)
        ssel = lax.shift_right_logical(bits, IB)
        bsel = jnp.where(ssel >= 0x8000, ssel - 0x8000, 0xFFFF - ssel)
        rsel = pltpu.bitcast(lax.shift_left(bsel, 16), F32)

        xs = None
        for j in range(TOPC):
            row = jnp.where(subl == j, oh_v[tile_s[j], 0:8, :].astype(F32), 0.0).astype(BF16)
            part = _nt(row, h2T_v[tile_s[j]])
            xs = part if xs is None else xs + part
        xs = xs.astype(BF16)

        for cp in cp_moe:
            cp.wait()
        gt = _r(_mm(xs, wg_v[...]))
        gt = _r(gt * _r(jax.nn.sigmoid(gt)))
        ut = _r(_mm(xs, wu_v[...]))
        y = _r(_nt((gt * ut).astype(BF16), wdT_v[...]))
        y = _r(y * _r(jax.nn.sigmoid(rsel[:, 0:1])))
        gy = y * gb_v[...]
        yT = jnp.transpose(jnp.concatenate([gy, jnp.zeros((LANES - 8, D), F32)], axis=0)).astype(BF16)

        for cp in o_copies(range(NT)):
            cp.wait()
        RQ = D // 4 // 16 * 16

        def patch_copy(j):
            c0 = pl.multiple_of(tile_s[j] * LANES, LANES)
            return pltpu.make_async_copy(h2T_v.at[j], oT_hbm.at[:, pl.ds(c0, LANES)], sem_p.at[j])

        def first_use(j):
            ok = tile_s[j] >= 0
            for k in range(j):
                ok = ok & (tile_s[j] != tile_s[k])
            return ok

        for j in range(TOPC):
            oh = oh_v[tile_s[j]]
            for q4 in range(4):
                rows = slice(q4 * RQ, D if q4 == 3 else (q4 + 1) * RQ)
                h2T_v[j, rows, :] = (accT_v[tile_s[j], rows, :] + _mm(yT[rows], oh)).astype(BF16)
            pl.when(first_use(j))(lambda j=j: patch_copy(j).start())
        for j in range(TOPC):
            pl.when(first_use(j))(lambda j=j: patch_copy(j).wait())

    return kernel


def make(BQ=512, UNR=4, OPOS='A1', QPOS='C6', vmem_mb=127):
    @jax.jit
    def fn(A_x, A_k_cache, A_v_cache, A_wq, A_wo, B_x, B_w_r, B_w_gate, B_w_up, B_w_down, c, w_mod):
        del B_x
        B, S, D = A_x.shape
        _, HKV, SK, _ = A_k_cache.shape
        F = B_w_gate.shape[1]
        REP = HQ // HKV
        NT = S // LANES
        NBLK = REP * BQ // 128
        any_spec = pl.BlockSpec(memory_space=pl.ANY)
        vmem_spec = pl.BlockSpec(memory_space=pltpu.VMEM)
        out = pl.pallas_call(
            _make_kernel(S, D, HKV, SK, F, BQ, UNR, OPOS, QPOS),
            out_shape=jax.ShapeDtypeStruct((D, S), BF16),
            in_specs=[any_spec, any_spec, any_spec, any_spec, any_spec, vmem_spec,
                      any_spec, any_spec, any_spec, vmem_spec, any_spec],
            out_specs=any_spec,
            scratch_shapes=[
                pltpu.VMEM((NT, D, LANES), BF16),
                pltpu.VMEM((HKV, SK, DH), BF16),
                pltpu.VMEM((HKV, SK, DH), BF16),
                pltpu.VMEM((HQ, D, DH), BF16),
                pltpu.VMEM((HQ, D, DH), BF16),
                pltpu.VMEM((D, F), BF16),
                pltpu.VMEM((D, F), BF16),
                pltpu.VMEM((D, F), BF16),
                pltpu.VMEM((D, 6 * D), BF16),
                pltpu.VMEM((S // 2, D), U32),
                pltpu.VMEM((REP, BQ // 2, DH), U32),
                pltpu.VMEM((REP, BQ // 2, DH), U32),
                pltpu.VMEM((NT, D, LANES), F32),
                pltpu.VMEM((NT, D, LANES), F32),
                pltpu.VMEM((4, D, LANES), F32),
                pltpu.VMEM((8, D), F32),
                pltpu.VMEM((NT, D, LANES), BF16),
                pltpu.VMEM((NT, LANES), F32),
                pltpu.VMEM((NT, LANES, LANES), BF16),
                pltpu.SemaphoreType.DMA((S // BQ,)),
                pltpu.SemaphoreType.DMA((2,)),
                pltpu.SemaphoreType.DMA((3,)),
                pltpu.SemaphoreType.DMA((2,)),
                pltpu.SemaphoreType.DMA(()),
                pltpu.SemaphoreType.DMA(()),
                pltpu.SemaphoreType.DMA((TOPC,)),
            ]
            + [pltpu.VMEM((1, 128, SK), F32)] * NBLK
            + [pltpu.VMEM((1, SK // LANES + 2, 64, LANES), U32)] * NBLK
            + [pltpu.VMEM((1, 128, LANES), F32)] * NBLK,
            compiler_params=pltpu.CompilerParams(vmem_limit_bytes=vmem_mb * 1024 * 1024),
        )(A_x.reshape(S, D).T, A_k_cache.reshape(HKV, SK, DH), A_v_cache.reshape(HKV, SK, DH),
          A_wq, A_wo.T, B_w_r, B_w_gate, B_w_up, B_w_down.T, c, w_mod)
        return out.T.reshape(B, S, D)

    return fn


pallas_adaLN_cond__gqa_block_cached__moe_arch_mod__prompt_kernel = make()
```
